```python
import os as _os
_os.environ.setdefault("JAX_PLATFORMS", "cpu")
import jax
import jax.numpy as jnp

def _softmax(x, axis=-1):
    return jax.nn.softmax(x, axis=axis)
def _gelu(x):
    return jax.nn.gelu(x, approximate=True)
def _silu(x):
    return jax.nn.silu(x)
def _sigmoid(x):
    return jax.nn.sigmoid(x)
def _layernorm(x, axis=-1, eps=1e-5):
    m = jnp.mean(x, axis=axis, keepdims=True)
    v = jnp.var(x, axis=axis, keepdims=True)
    return (x - m) / jnp.sqrt(v + eps)
def _scatter_add(tgt, idx, src, axis=0):
    return tgt.at[idx].add(src)
def _segment_sum(src, seg, n):
    return jax.ops.segment_sum(src, seg, n)
class _Rng:
    def __init__(self, key):
        self._k = key
    def _next(self):
        self._k, sub = jax.random.split(self._k)
        return sub
    def normal(self, shape):
        return jax.random.normal(self._next(), shape, dtype=jnp.bfloat16)
    def randint(self, lo, hi, shape):
        return jax.random.randint(self._next(), shape, lo, hi, dtype=jnp.int32)
    def uniform(self, shape, lo=0.0, hi=1.0):
        return jax.random.uniform(self._next(), shape, jnp.bfloat16, lo, hi)
    def permutation(self, n):
        return jax.random.permutation(self._next(), n)


kernel_name = 'standalone__gqa_block_cached__near_ridge'

def setup_inputs():
    _rng = _Rng(jax.random.key(int.from_bytes(__import__("os").urandom(4), "little")))
    _w = (lambda a: (lambda t: t.astype(jnp.bfloat16) if jnp.issubdtype(t.dtype, jnp.floating) else t)(jnp.asarray(a)))
    B, Sq, D = 8, 64, 512
    Hq, Hkv, Sk, Dh = 32, 8, 64, 128
    assert Hq % Hkv == 0, (Hq, Hkv)
    return {
        "x": _w((lambda *s: _rng.normal(s) * 0.8)(B, Sq, D)),
        "k_cache": _w((lambda *s: _rng.normal(s) * 0.8)(B, Hkv, Sk, Dh)),
        "v_cache": _w((lambda *s: _rng.normal(s) * 0.05)(B, Hkv, Sk, Dh)),
        "wq": _w((lambda *s: _rng.normal(s) * 0.8)(D, Hq * Dh) * (D ** -0.5)),
        "wo": _w((lambda *s: _rng.normal(s) * 0.05)(Hq * Dh, D) * ((Hq * Dh) ** -0.5)),
    }

def reference(x, k_cache, v_cache, wq, wo):
    B, Sq, D = x.shape
    Hq, Dh = 32, 128
    Hkv = k_cache.shape[1]
    rep = Hq // Hkv
    q = (lambda x, *d: x.transpose(*d))((x @ wq).reshape(B, Sq, Hq, Dh), 0, 2, 1, 3)
    k = jnp.repeat(k_cache, rep, axis=1)
    v = jnp.repeat(v_cache, rep, axis=1)
    scores = jnp.einsum("bhqd,bhkd->bhqk", q, k) * (Dh ** -0.5)
    p = _softmax(scores, axis=-1)
    o = jnp.einsum("bhqk,bhkd->bhqd", p, v)
    return (lambda x, *d: x.transpose(*d))(o, 0, 2, 1, 3).reshape(B, Sq, Hq * Dh) @ wo
```

```python
import functools

import jax
import jax.numpy as jnp
import jax.experimental.pallas as pl
import jax.experimental.pallas.tpu as pltpu

_HQ = 32
_DH = 128


def _kernel(x_ref, k_ref, v_ref, wq_ref, wo_ref, o_ref, acc_ref, oh_ref, *,
            B, Sq, rep, Sk, scale):
    g = pl.program_id(0)

    @pl.when(g == 0)
    def _():
        acc_ref[...] = jnp.zeros_like(acc_ref)

    q = jnp.dot(x_ref[...], wq_ref[...], preferred_element_type=jnp.float32)
    q = q.astype(jnp.bfloat16)

    for b in range(B):
        qb = q[b * Sq:(b + 1) * Sq, :]
        qs = jnp.concatenate(
            [qb[:, h * _DH:(h + 1) * _DH] for h in range(rep)], axis=0)
        kb = k_ref[b]
        vb = v_ref[b]
        s = jax.lax.dot_general(
            qs, kb, (((1,), (1,)), ((), ())),
            preferred_element_type=jnp.float32)
        m = jnp.max(s, axis=-1, keepdims=True)
        p = jnp.exp((s - m) * scale)
        l = jnp.sum(p, axis=-1, keepdims=True)
        p = (p / l).astype(jnp.bfloat16)
        o = jnp.dot(p, vb, preferred_element_type=jnp.float32)
        o = o.astype(jnp.bfloat16)
        ocat = jnp.concatenate(
            [o[h * Sq:(h + 1) * Sq, :] for h in range(rep)], axis=1)
        oh_ref[b * Sq:(b + 1) * Sq, :] = ocat

    acc_ref[...] += jnp.dot(oh_ref[...], wo_ref[...],
                            preferred_element_type=jnp.float32)

    @pl.when(g == pl.num_programs(0) - 1)
    def _():
        o_ref[...] = acc_ref[...].astype(o_ref.dtype)


@jax.jit
def pallas_standalone__gqa_block_cached__near_ridge_kernel(
    x: jax.Array,
    k_cache: jax.Array,
    v_cache: jax.Array,
    wq: jax.Array,
    wo: jax.Array,
):
    B, Sq, D = x.shape
    _, Hkv, Sk, Dh = k_cache.shape
    rep = _HQ // Hkv
    M = B * Sq
    x2 = x.reshape(M, D)
    gw = rep * Dh

    kernel = functools.partial(
        _kernel, B=B, Sq=Sq, rep=rep, Sk=Sk, scale=float(Dh) ** -0.5)

    out = pl.pallas_call(
        kernel,
        grid=(Hkv,),
        in_specs=[
            pl.BlockSpec((M, D), lambda g: (0, 0)),
            pl.BlockSpec((B, None, Sk, Dh), lambda g: (0, g, 0, 0)),
            pl.BlockSpec((B, None, Sk, Dh), lambda g: (0, g, 0, 0)),
            pl.BlockSpec((D, gw), lambda g: (0, g)),
            pl.BlockSpec((gw, D), lambda g: (g, 0)),
        ],
        out_specs=pl.BlockSpec((M, D), lambda g: (0, 0)),
        out_shape=jax.ShapeDtypeStruct((M, D), x.dtype),
        scratch_shapes=[
            pltpu.VMEM((M, D), jnp.float32),
            pltpu.VMEM((M, gw), jnp.bfloat16),
        ],
        compiler_params=pltpu.CompilerParams(
            dimension_semantics=("arbitrary",),
            vmem_limit_bytes=64 * 1024 * 1024,
        ),
    )(x2, k_cache, v_cache, wq, wo)
    return out.reshape(B, Sq, D)
```

```python
import functools

import jax
import jax.numpy as jnp
import jax.experimental.pallas as pl
import jax.experimental.pallas.tpu as pltpu

_HQ = 32
_LOG2E = 1.4426950408889634

_K_CHUNKS = 4
_OUT_BOUNDS = (0, 256, 384, 448, 512)
_Q_PIECES = 4
_BARRIERS = frozenset({(1, "qk"), (1, "qp"), (1, "pv"), (2, "qp"), (3, "qp"), (5, "qp")})


def _kernel(x_hbm, k_hbm, v_hbm, wq_hbm, wo_hbm, out_hbm,
            x_v, wq_v, wo_v, k_v, v_v, q_ref, oh_ref, oh2_ref, acc_ref, sems, *out_stage,
            B, Sq, rep, Dh, D, G, scale):
    gw = rep * Dh
    kcw = D // _K_CHUNKS
    OB = _OUT_BOUNDS
    NOC = len(OB) - 1
    f32 = jnp.float32
    bf16 = jnp.bfloat16

    n_sem = [0]

    def copy(src, dst):
        cp = pltpu.make_async_copy(src, dst, sems.at[n_sem[0]])
        n_sem[0] += 1
        return cp

    x_cp = [copy(x_hbm.at[:, pl.ds(kc * kcw, kcw)], x_v.at[kc]) for kc in range(_K_CHUNKS)]
    wq0_cp = [copy(wq_hbm.at[pl.ds(kc * kcw, kcw), pl.ds(0, gw)],
                   wq_v.at[0, pl.ds(kc * kcw, kcw), :]) for kc in range(_K_CHUNKS)]
    k_cp = [copy(k_hbm.at[:, g], k_v.at[g]) for g in range(G)]
    v_cp = [copy(v_hbm.at[:, g], v_v.at[g]) for g in range(G)]
    wq_cp = [None] + [copy(wq_hbm.at[:, pl.ds(g * gw, gw)], wq_v.at[g]) for g in range(1, G)]
    wo_cp = [copy(wo_hbm.at[pl.ds(g * gw, gw), :], wo_v.at[g]) for g in range(G)]
    out_cp = [copy(out_stage[oc], out_hbm.at[pl.ds(OB[oc], OB[oc + 1] - OB[oc]), :])
              for oc in range(NOC)]

    def x_full():
        return jnp.concatenate([x_v[kc] for kc in range(_K_CHUNKS)], axis=1)

    def qproj0_chunk(kc):
        part = jnp.dot(x_v[kc], wq_v[0, kc * kcw:(kc + 1) * kcw, :], preferred_element_type=f32)
        if kc == 0:
            acc_ref[...] = part
        elif kc < _K_CHUNKS - 1:
            acc_ref[...] += part
        else:
            q_ref[...] = (acc_ref[...] + part).astype(bf16)

    def qproj_piece(xf, g, j):
        w = gw // _Q_PIECES
        q = jnp.dot(xf, wq_v[g, :, j * w:(j + 1) * w], preferred_element_type=f32)
        q_ref[:, j * w:(j + 1) * w] = q.astype(bf16)

    def qk(g):
        sts = []
        for b in range(B):
            qs = jnp.concatenate(
                [q_ref[b * Sq:(b + 1) * Sq, h * Dh:(h + 1) * Dh] for h in range(rep)], axis=0)
            sts.append(jax.lax.dot_general(k_v[g, b], qs, (((1,), (1,)), ((), ())),
                                           preferred_element_type=f32))
        return sts

    def softmax_t(st):
        m = jnp.max(st, axis=0, keepdims=True)
        p = jnp.exp2((st - m) * (scale * _LOG2E))
        l = jnp.sum(p, axis=0, keepdims=True)
        return (p * (1.0 / l)).astype(bf16)

    def softmax_and_qproj(sts, g):
        xf = x_full()
        per = B // _Q_PIECES
        pts = []
        for j in range(_Q_PIECES):
            for b in range(j * per, (j + 1) * per):
                pts.append(softmax_t(sts[b]))
            qproj_piece(xf, g, j)
        return pts

    def pv(pts, g, oh):
        for b in range(B):
            o = jax.lax.dot_general(pts[b], v_v[g, b], (((0,), (0,)), ((), ())),
                                    preferred_element_type=f32).astype(bf16)
            oh[b * Sq:(b + 1) * Sq, :] = jnp.concatenate(
                [o[h * Sq:(h + 1) * Sq, :] for h in range(rep)], axis=1)

    def oproj(oh, g, first):
        r = jnp.dot(oh[...], wo_v[g], preferred_element_type=f32)
        if first:
            acc_ref[...] = r
        else:
            acc_ref[...] += r

    def oproj_final(oh, g):
        for oc in range(NOC):
            rows = slice(OB[oc], OB[oc + 1])
            r = jnp.dot(oh[rows, :], wo_v[g], preferred_element_type=f32)
            out_stage[oc][...] = (acc_ref[rows, :] + r).astype(out_stage[oc].dtype)
            out_cp[oc].start()

    val = {}

    def do_qk(g):
        val["sts"] = qk(g)

    def do_sm_qp(g):
        val["pts"] = softmax_and_qproj(val["sts"], g)

    def do_sm():
        val["pts"] = [softmax_t(s) for s in val["sts"]]

    def do_pv(g, oh):
        pv(val["pts"], g, oh)

    P = functools.partial
    ops = []
    for kc in range(_K_CHUNKS):
        ops.append((0, "qp0", [x_cp[kc], wq0_cp[kc]], P(qproj0_chunk, kc)))
    for s in range(1, G + 1):
        g = s - 1
        ops.append((s, "qk", [k_cp[g]], P(do_qk, g)))
        if s < G:
            oh = oh2_ref if s == G - 1 else oh_ref
            ops.append((s, "qp", [wq_cp[s]], P(do_sm_qp, s)))
            ops.append((s, "pv", [v_cp[g]], P(do_pv, g, oh)))
            if s < G - 1:
                ops.append((s, "op", [wo_cp[g]], P(oproj, oh_ref, g, g == 0)))
        else:
            ops.append((s, "op_prev", [wo_cp[g - 1]], P(oproj, oh2_ref, g - 1, False)))
            ops.append((s, "sm", [], do_sm))
            ops.append((s, "pv", [v_cp[g]], P(do_pv, g, oh_ref)))
            ops.append((s, "op", [wo_cp[g]], P(oproj_final, oh_ref, g)))

    wait_at = [[] for _ in ops]
    seen = set()
    last_barrier = None
    for i, (s, kind, needs, _) in enumerate(ops):
        if s == 0 or (s, kind) in _BARRIERS:
            last_barrier = i
        for cp in needs:
            if id(cp) not in seen:
                seen.add(id(cp))
                wait_at[last_barrier].append(cp)

    for kc in range(_K_CHUNKS):
        x_cp[kc].start()
        wq0_cp[kc].start()
    for g in range(G):
        k_cp[g].start()
        if g + 1 < G:
            wq_cp[g + 1].start()
        v_cp[g].start()
        wo_cp[g].start()

    n_waited = 0
    for i, (_, _, _, thunk) in enumerate(ops):
        for cp in wait_at[i]:
            cp.wait()
            n_waited += 1
        thunk()
    for cp in out_cp:
        cp.wait()
    assert n_waited == 2 * _K_CHUNKS + 4 * G - 1


@jax.jit
def pallas_standalone__gqa_block_cached__near_ridge_kernel(
    x: jax.Array,
    k_cache: jax.Array,
    v_cache: jax.Array,
    wq: jax.Array,
    wo: jax.Array,
):
    B, Sq, D = x.shape
    _, G, Sk, Dh = k_cache.shape
    rep = _HQ // G
    M = B * Sq
    gw = rep * Dh
    assert _HQ % G == 0 and G >= 3
    assert wq.shape == (D, _HQ * Dh) and wo.shape == (_HQ * Dh, D)
    assert D % (_K_CHUNKS * 128) == 0 and Dh % 128 == 0 and gw % (_Q_PIECES * 128) == 0
    assert B % _Q_PIECES == 0 and Sq % 16 == 0 and Sk % 16 == 0
    assert _OUT_BOUNDS[0] == 0 and _OUT_BOUNDS[-1] == M

    kernel = functools.partial(_kernel, B=B, Sq=Sq, rep=rep, Dh=Dh, D=D, G=G,
                               scale=float(Dh) ** -0.5)
    n_out_chunks = len(_OUT_BOUNDS) - 1
    n_sem = 2 * _K_CHUNKS + 4 * G - 1 + n_out_chunks
    bf16 = jnp.bfloat16
    hbm = pl.BlockSpec(memory_space=pl.ANY)
    out = pl.pallas_call(
        kernel,
        in_specs=[hbm] * 5,
        out_specs=hbm,
        out_shape=jax.ShapeDtypeStruct((M, D), x.dtype),
        scratch_shapes=[
            pltpu.VMEM((_K_CHUNKS, M, D // _K_CHUNKS), bf16),
            pltpu.VMEM((G, D, gw), bf16),
            pltpu.VMEM((G, gw, D), bf16),
            pltpu.VMEM((G, B, Sk, Dh), bf16),
            pltpu.VMEM((G, B, Sk, Dh), bf16),
            pltpu.VMEM((M, gw), bf16),
            pltpu.VMEM((M, gw), bf16),
            pltpu.VMEM((M, gw), bf16),
            pltpu.VMEM((M, D), jnp.float32),
            pltpu.SemaphoreType.DMA((n_sem,)),
        ] + [pltpu.VMEM((_OUT_BOUNDS[i + 1] - _OUT_BOUNDS[i], D), x.dtype)
             for i in range(n_out_chunks)],
        compiler_params=pltpu.CompilerParams(vmem_limit_bytes=64 * 1024 * 1024),
    )(x.reshape(M, D), k_cache, v_cache, wq, wo)
    return out.reshape(B, Sq, D)
```
